```python
import os as _os
_os.environ.setdefault("JAX_PLATFORMS", "cpu")
import jax
import jax.numpy as jnp

def _softmax(x, axis=-1):
    return jax.nn.softmax(x, axis=axis)
def _gelu(x):
    return jax.nn.gelu(x, approximate=True)
def _silu(x):
    return jax.nn.silu(x)
def _sigmoid(x):
    return jax.nn.sigmoid(x)
def _layernorm(x, axis=-1, eps=1e-5):
    m = jnp.mean(x, axis=axis, keepdims=True)
    v = jnp.var(x, axis=axis, keepdims=True)
    return (x - m) / jnp.sqrt(v + eps)
def _scatter_add(tgt, idx, src, axis=0):
    return tgt.at[idx].add(src)
def _segment_sum(src, seg, n):
    return jax.ops.segment_sum(src, seg, n)
class _Rng:
    def __init__(self, key):
        self._k = key
    def _next(self):
        self._k, sub = jax.random.split(self._k)
        return sub
    def normal(self, shape):
        return jax.random.normal(self._next(), shape, dtype=jnp.bfloat16)
    def randint(self, lo, hi, shape):
        return jax.random.randint(self._next(), shape, lo, hi, dtype=jnp.int32)
    def uniform(self, shape, lo=0.0, hi=1.0):
        return jax.random.uniform(self._next(), shape, jnp.bfloat16, lo, hi)
    def permutation(self, n):
        return jax.random.permutation(self._next(), n)


kernel_name = 'concat_heads__ssm_conv_h3__sliding_block__prompt'

def setup_inputs():
    _rng = _Rng(jax.random.key(int.from_bytes(__import__("os").urandom(4), "little")))
    _w = (lambda a: (lambda t: t.astype(jnp.bfloat16) if jnp.issubdtype(t.dtype, jnp.floating) else t)(jnp.asarray(a)))
    def _A_setup():
        B, S, D = 1, 2048, 512
        ks = 4
        return {
            "q": _w((lambda *s: _rng.normal(s) * 0.05)(B, S, D)),
            "k": _w((lambda *s: _rng.normal(s) * 0.2)(B, S, D)),
            "v": _w((lambda *s: _rng.normal(s) * 0.2)(B, S, D)),
            "shift_k": _w((lambda *s: _rng.normal(s) * 0.2)(D, ks) * 0.5),
            "ssm_k": _w((lambda *s: _rng.normal(s) * 0.2)(D, S) * (1.0 / S ** 0.5)),
            "ssm_D": _w((lambda *s: _rng.normal(s) * 0.2)(D)),
        }
    _A_in = _A_setup()

    def _B_setup():
        B, S, D = 1, 2048, 512
        return {
            "x": _w((lambda *s: _rng.normal(s) * 0.2)(B, S, D)),
            "wqkv": _w((lambda *s: _rng.normal(s) * 0.2)(D, 3 * D)),
            "wo": _w((lambda *s: _rng.normal(s) * 0.05)(D, D)),
        }
    _B_in = _B_setup()

    return {
        "A_q": _A_in["q"],
        "A_k": _A_in["k"],
        "A_v": _A_in["v"],
        "A_shift_k": _A_in["shift_k"],
        "A_ssm_k": _A_in["ssm_k"],
        "A_ssm_D": _A_in["ssm_D"],
        "B_x": _B_in["x"],
        "B_wqkv": _B_in["wqkv"],
        "B_wo": _B_in["wo"],
    }

def reference(A_q, A_k, A_v, A_shift_k, A_ssm_k, A_ssm_D, B_x, B_wqkv, B_wo):
    def _A_ref(q, k, v, shift_k, ssm_k, ssm_D):
        B, S, D = q.shape
        ks = shift_k.shape[-1]
        k_pad = jnp.pad(k, ((0, 0), (ks - 1, 0), (0, 0)))
        k_shift = jnp.zeros_like(k)
        for t in range(ks):
            k_shift = k_shift + k_pad[:, t:t + S, :] * shift_k[:, ks - 1 - t][None, None, :]
        kv = k_shift * v
        L = 2 * S
        kv_pad = jnp.pad(kv, ((0, 0), (0, S), (0, 0)))
        kf_pad = jnp.pad(ssm_k, ((0, 0), (0, S)))
        kv_f = (lambda x, axes=(-2,-1): jnp.fft.rfft2(x.astype(jnp.float32), axes=axes))(kv_pad[:, None, :, :], axes=(1, 2))
        kf_f = (lambda x, axes=(-2,-1): jnp.fft.rfft2(x.astype(jnp.float32), axes=axes))(kf_pad[:, None, :], axes=(1, 2))
        kf_f = (lambda x, *d: x.transpose(*d))(kf_f, 1, 2, 0)
        y_f = kv_f * kf_f[None, :, :, :]
        y = (lambda x, s, axes=(-2,-1): jnp.fft.irfft2(x, s=s, axes=axes).astype(jnp.bfloat16))(y_f, (1, L), axes=(1, 2))[:, 0, :S, :]
        y = y + kv * ssm_D[None, None, :]
        return q * y

    def _B_ref(x, wqkv, wo):
        B, S, D = x.shape
        H = 32; Dh = D // H; W = 256
        qkv = (lambda x, *d: x.transpose(*d))((x @ wqkv).reshape(B, S, 3, H, Dh), 2, 0, 3, 1, 4)
        q, k, v = qkv[0], qkv[1], qkv[2]
        scores = jnp.einsum("bhqd,bhkd->bhqk", q, k) * (Dh ** -0.5)
        idx = jnp.arange(S)
        mask = (idx[:, None] - idx[None, :] >= 0) & (idx[:, None] - idx[None, :] < W)
        scores = jnp.where(mask[None, None], scores, -1e9)
        p = _softmax(scores, axis=-1)
        o = jnp.einsum("bhqk,bhkd->bhqd", p, v)
        return (lambda x, *d: x.transpose(*d))(o, 0, 2, 1, 3).reshape(B, S, D) @ wo

    a = _A_ref(A_q, A_k, A_v, A_shift_k, A_ssm_k, A_ssm_D)
    b = _B_ref(B_x, B_wqkv, B_wo)
    return jnp.concatenate([a, b], axis=-1)
```

```python
import functools

import jax
import jax.numpy as jnp
import numpy as np
import jax.experimental.pallas as pl
import jax.experimental.pallas.tpu as pltpu

S, D, H, DH, W = 2048, 512, 32, 16, 256
T = 128
NB = S // T
F32, BF16 = jnp.float32, jnp.bfloat16


def _dft_consts():
    f = np.arange(128)[:, None] + 0.5
    n = np.arange(128)[None, :]
    ang = 2.0 * np.pi * f * n / 256.0
    fwd = np.concatenate([np.cos(ang), -np.sin(ang)], axis=0)
    inv = np.concatenate([np.cos(ang).T, -np.sin(ang).T], axis=1) / 128.0
    return fwd.astype(np.float32), inv.astype(np.float32)


def _nt(a, b):
    return jax.lax.dot_general(a, b, (((1,), (1,)), ((), ())), preferred_element_type=F32)


def _nn(a, b):
    return jnp.dot(a, b, preferred_element_type=F32)


PAD = 8
VARIANTS = ((0, 2, 2, True), (2, 8, 8, False), (8, 12, 12, False), (12, 16, 16, False))
AHEAD = 6


def _group(i, nt, edge, refs, g, acc):
    (q_ref, k_ref, v_ref, sk_ref, h_ref, sd_ref, x_ref, w_ref, wo_ref, ff_ref, fi_ref,
     o_ref, wqt, wvt, wos, skt, kbuf, xf, hf, hprev, k_s, vt_s, oacc) = refs
    gl = pl.ds(pl.multiple_of(g * 128, 128), 128)
    x = x_ref[...]
    xs = jnp.concatenate([x[64:128], x[0:64]], axis=0)
    pre = {}
    def hist(r):
        a = b = None
        for j in range(nt):
            xr = xf[g, i + PAD - j, r:r + 16, :]; xi = xf[g, i + PAD - j, 128 + r:144 + r, :]
            hr = hf[g, j, r:r + 16, :]; hi = hf[g, j, 128 + r:144 + r, :]
            a = xr * hr - xi * hi if a is None else a + xr * hr - xi * hi
            b = xr * hi + xi * hr if b is None else b + xr * hi + xi * hr
        pre[r] = (0.0, 0.0) if a is None else (a, b)

    qe = _nt(wqt[g, 0:64, :], x)
    qo = _nt(wqt[g, 64:128, :], xs)
    k_s[g, i + 2] = _nn(x, w_ref[:, pl.ds(pl.multiple_of(D + g * 128, 128), 128)]).astype(BF16)
    vt_s[g, i + 2] = _nt(wvt[g], x).astype(BF16)

    kbuf[g, 0:8, :] = kbuf[g, T:T + 8, :]
    kbuf[g, 8:8 + T, :] = k_ref[:, gl].astype(F32)
    ks = kbuf[g, 8:8 + T, :] * skt[0:1, gl]
    for j in range(1, 4):
        ks = ks + kbuf[g, 8 - j:8 - j + T, :] * skt[j:j + 1, gl]
    kv = (ks * v_ref[:, gl].astype(F32)).astype(BF16)
    xx = _nn(ff_ref[...], kv)
    hh = _nt(ff_ref[...], h_ref[gl, :])
    sgn = (1 - 2 * (jax.lax.broadcasted_iota(jnp.int32, (128, 128), 0) & 1)).astype(F32)
    hf[g, i, 0:128, :] = hh[0:128] - sgn * hprev[g, 128:256]
    hf[g, i, 128:256, :] = hh[128:256] + sgn * hprev[g, 0:128]
    hprev[g] = hh
    xf[g, i + PAD] = xx

    def mac(r):
        hist(r)
        return pre[r][0].astype(BF16), pre[r][1].astype(BF16)

    lo = jax.lax.broadcasted_iota(jnp.int32, (16, 128), 1) < 64
    zero16 = jnp.zeros((16, 128), BF16)
    z = jnp.zeros((64, 128), BF16)
    qi = jax.lax.broadcasted_iota(jnp.int32, (64, 128), 1) & 63
    kj = jax.lax.broadcasted_iota(jnp.int32, (64, 128), 0)

    def qk(u):
        p, half = divmod(u, 2)
        e = qe[p * 16:(p + 1) * 16]; o = qo[p * 16:(p + 1) * 16]
        if half == 0:
            e = jnp.where(lo, e, 0.0); o = jnp.where(lo, 0.0, o)
            kk = [k_s[g, i], k_s[g, i + 1], k_s[g, i + 2, 0:64]]
        else:
            e = jnp.where(lo, 0.0, e); o = jnp.where(lo, o, 0.0)
            kk = [k_s[g, i, 64:128], k_s[g, i + 1], k_s[g, i + 2]]
        rhs = jnp.concatenate([zero16] * (2 * p) + [e.astype(BF16), o.astype(BF16)]
                              + [zero16] * (6 - 2 * p), axis=0)
        return _nn(jnp.concatenate(kk, axis=0), rhs)

    def smax(u, s):
        p, half = divmod(u, 2)
        parts = [s[c * 64:(c + 1) * 64] for c in range(5)]
        parts[0] = jnp.where(kj > qi, parts[0], -1e30)
        parts[4] = jnp.where(kj <= qi, parts[4], -1e30)
        if edge:
            for c in range(4):
                parts[c] = jnp.where(i * 2 + half + c >= 4, parts[c], -1e30)
        m = parts[0]
        for sc in parts[1:]:
            m = jnp.maximum(m, sc)
        return parts, jnp.max(m, axis=0, keepdims=True)

    ones = jnp.ones((16, 384), BF16)

    def pv(u, pm):
        parts, m = pm
        p, half = divmod(u, 2)
        ps = [jnp.exp2(sc - m) for sc in parts]
        pb = [z] * half + [t.astype(BF16) for t in ps] + [z] * (1 - half)
        vt = jnp.concatenate([vt_s[g, i + c, p * 32:(p + 1) * 32, :] for c in range(3)], axis=1)
        return _nn(jnp.concatenate([vt, ones], axis=0), jnp.concatenate(pb, axis=0))

    ss, mm, raw, res, ys = {}, {}, {}, [], []
    for t in range(8 + AHEAD + 1):
        if t < 8:
            ss[t] = qk(t)
        if 0 <= t - AHEAD < 8:
            raw[t - AHEAD] = pv(t - AHEAD, mm.pop(t - AHEAD))
        if 0 <= t - 1 < 8:
            mm[t - 1] = smax(t - 1, ss.pop(t - 1))
        if t < 8:
            ys.append(mac(t * 16))
        if 0 <= t - AHEAD - 1 < 8:
            r = raw.pop(t - AHEAD - 1)
            inv = 1.0 / r[32:40]
            res.append(r[0:32] * jnp.concatenate([inv] * 4, axis=0))
    y = _nn(fi_ref[...], jnp.concatenate([t[0] for t in ys] + [t[1] for t in ys], axis=0))
    ote = [jnp.where(lo, res[2 * p][0:16], res[2 * p + 1][0:16]) for p in range(4)]
    oto = [jnp.where(lo, res[2 * p + 1][16:32], res[2 * p][16:32]) for p in range(4)]
    oacc[g] = jnp.concatenate(ote + oto, axis=0)
    y = y + kv.astype(F32) * sd_ref[:, gl].astype(F32)
    o_ref[:, gl] = (q_ref[:, gl].astype(F32) * y).astype(BF16)
    return acc


def _kernel(*refs):
    (q_ref, k_ref, v_ref, sk_ref, h_ref, sd_ref, x_ref, w_ref, wo_ref, ff_ref, fi_ref,
     o_ref, wqt, wvt, wos, skt, kbuf, xf, hf, hprev, k_s, vt_s, oacc) = refs
    i = pl.program_id(0)

    @pl.when(i == 0)
    def _():
        skt[...] = sk_ref[...].astype(F32).T

        def init(g, c):
            gl = pl.ds(pl.multiple_of(g * 128, 128), 128)
            wq = (w_ref[:, gl].astype(F32) * (DH ** -0.5 * 1.4426950408889634)).T
            wvt[g] = w_ref[:, pl.ds(pl.multiple_of(2 * D + g * 128, 128), 128)].astype(F32).T.astype(BF16)
            for h in range(8):
                r = (h % 2) * 64 + (h // 2) * 16
                wqt[g, r:r + 16, :] = wq[h * 16:(h + 1) * 16, :].astype(BF16)
                wos[pl.ds(pl.multiple_of((h % 2) * 256 + g * 64 + (h // 2) * 16, 16), 16), :] = wo_ref[pl.ds(pl.multiple_of(g * 128 + h * 16, 16), 16), :]
            kbuf[g, T:T + 8, :] = jnp.zeros((8, 128), F32)
            hprev[g] = jnp.zeros((256, 128), F32)
            for c2 in range(2):
                k_s[g, c2] = jnp.zeros((128, 128), BF16)
                vt_s[g, c2] = jnp.zeros((128, 128), BF16)
            return c
        jax.lax.fori_loop(0, 4, init, 0)

        def init2(n, c):
            xf[n // 8, n % 8] = jnp.zeros((256, 128), F32)
            hf[n // 8, (n % 8) * 2] = jnp.zeros((256, 128), F32)
            hf[n // 8, (n % 8) * 2 + 1] = jnp.zeros((256, 128), F32)
            return c
        jax.lax.fori_loop(0, 32, init2, 0)

    for lo_, hi_, nt, edge in VARIANTS:
        @pl.when(jnp.logical_and(i >= lo_, i < hi_))
        def _(nt=nt, edge=edge):
            jax.lax.fori_loop(0, 4, functools.partial(_group, i, nt, edge, refs), 0)
    oe = jnp.concatenate([oacc[g, 0:64] for g in range(4)], axis=0).T.astype(BF16)
    oo = jnp.concatenate([oacc[g, 64:128] for g in range(4)], axis=0).T.astype(BF16)
    oo = jnp.concatenate([oo[64:128], oo[0:64]], axis=0)
    o_ref[:, D:2 * D] = _nn(jnp.concatenate([oe, oo], axis=1), wos[...]).astype(BF16)


@jax.jit
def pallas_concat_heads__ssm_conv_h3__sliding_block__prompt_kernel(
    A_q, A_k, A_v, A_shift_k, A_ssm_k, A_ssm_D, B_x, B_wqkv, B_wo,
):
    fwd, inv = _dft_consts()
    row = pl.BlockSpec((None, T, D), lambda i: (0, i, 0))
    full = lambda shp: pl.BlockSpec(shp, lambda i: (0,) * len(shp))
    return pl.pallas_call(
        _kernel,
        grid=(NB,),
        in_specs=[row, row, row, full((D, 4)), pl.BlockSpec((D, T), lambda i: (0, i)),
                  full((1, D)), row, full((D, 3 * D)), full((D, D)),
                  full((256, 128)), full((128, 256))],
        out_specs=pl.BlockSpec((None, T, 2 * D), lambda i: (0, i, 0)),
        out_shape=jax.ShapeDtypeStruct((1, S, 2 * D), BF16),
        scratch_shapes=[
            pltpu.VMEM((4, 128, D), BF16), pltpu.VMEM((4, 128, D), BF16),
            pltpu.VMEM((D, D), BF16), pltpu.VMEM((4, D), F32),
            pltpu.VMEM((4, T + 8, 128), F32), pltpu.VMEM((4, NB + PAD, 256, 128), F32),
            pltpu.VMEM((4, NB, 256, 128), F32), pltpu.VMEM((4, 256, 128), F32),
            pltpu.VMEM((4, NB + 2, 128, 128), BF16), pltpu.VMEM((4, NB + 2, 128, 128), BF16),
            pltpu.VMEM((4, 128, 128), F32),
        ],
        compiler_params=pltpu.CompilerParams(
            dimension_semantics=("arbitrary",), vmem_limit_bytes=100 * 1024 * 1024),
    )(A_q, A_k, A_v, A_shift_k, A_ssm_k, A_ssm_D.reshape(1, D), B_x, B_wqkv, B_wo,
      jnp.asarray(fwd, BF16), jnp.asarray(inv, BF16))
```
